```python
import os as _os
_os.environ.setdefault("JAX_PLATFORMS", "cpu")
import jax
import jax.numpy as jnp

def _softmax(x, axis=-1):
    return jax.nn.softmax(x, axis=axis)
def _gelu(x):
    return jax.nn.gelu(x, approximate=True)
def _silu(x):
    return jax.nn.silu(x)
def _sigmoid(x):
    return jax.nn.sigmoid(x)
def _layernorm(x, axis=-1, eps=1e-5):
    m = jnp.mean(x, axis=axis, keepdims=True)
    v = jnp.var(x, axis=axis, keepdims=True)
    return (x - m) / jnp.sqrt(v + eps)
def _scatter_add(tgt, idx, src, axis=0):
    return tgt.at[idx].add(src)
def _segment_sum(src, seg, n):
    return jax.ops.segment_sum(src, seg, n)
class _Rng:
    def __init__(self, key):
        self._k = key
    def _next(self):
        self._k, sub = jax.random.split(self._k)
        return sub
    def normal(self, shape):
        return jax.random.normal(self._next(), shape, dtype=jnp.bfloat16)
    def randint(self, lo, hi, shape):
        return jax.random.randint(self._next(), shape, lo, hi, dtype=jnp.int32)
    def uniform(self, shape, lo=0.0, hi=1.0):
        return jax.random.uniform(self._next(), shape, jnp.bfloat16, lo, hi)
    def permutation(self, n):
        return jax.random.permutation(self._next(), n)


kernel_name = 'sequential_preLN__softmax_full_mha__swiglu_ffn__prompt'

def setup_inputs():
    _rng = _Rng(jax.random.key(int.from_bytes(__import__("os").urandom(4), "little")))
    _w = (lambda a: (lambda t: t.astype(jnp.bfloat16) if jnp.issubdtype(t.dtype, jnp.floating) else t)(jnp.asarray(a)))
    def _A_setup():
        B, S, D = 1, 2048, 512
        return {
            "x": _w((lambda *s: _rng.normal(s) * 0.05)(B, S, D)),
            "wqkv": _w((lambda *s: _rng.normal(s) * 0.05)(D, 3 * D)),
            "wo": _w((lambda *s: _rng.normal(s) * 0.05)(D, D)),
        }
    _A_in = _A_setup()

    def _B_setup():
        B, S, D, F = 1, 2048, 512, 1792
        return {
            "x": _w((lambda *s: _rng.normal(s) * 0.05)(B, S, D)),
            "w_gate": _w((lambda *s: _rng.normal(s) * 0.05)(D, F)),
            "w_up": _w((lambda *s: _rng.normal(s) * 0.05)(D, F)),
            "w_down": _w((lambda *s: _rng.normal(s) * 0.05)(F, D)),
        }
    _B_in = _B_setup()

    return {
        "A_x": _A_in["x"],
        "A_wqkv": _A_in["wqkv"],
        "A_wo": _A_in["wo"],
        "B_x": _B_in["x"],
        "B_w_gate": _B_in["w_gate"],
        "B_w_up": _B_in["w_up"],
        "B_w_down": _B_in["w_down"],
    }

def reference(A_x, A_wqkv, A_wo, B_x, B_w_gate, B_w_up, B_w_down):
    def _A_ref(x, wqkv, wo):
        B, S, D = x.shape
        H = 32; Dh = D // H
        qkv = (lambda x, *d: x.transpose(*d))((x @ wqkv).reshape(B, S, 3, H, Dh), 2, 0, 3, 1, 4)
        q, k, v = qkv[0], qkv[1], qkv[2]
        scale = Dh ** -0.5
        scores = jnp.einsum("bhqd,bhkd->bhqk", q, k) * scale
        p = _softmax(scores, axis=-1)
        o = jnp.einsum("bhqk,bhkd->bhqd", p, v)
        return (lambda x, *d: x.transpose(*d))(o, 0, 2, 1, 3).reshape(B, S, D) @ wo

    def _B_ref(x, w_gate, w_up, w_down):
        g = _silu(x @ w_gate)
        u = x @ w_up
        return (g * u) @ w_down

    x = A_x
    h = x + _A_ref(_layernorm(x, axis=-1), A_wqkv, A_wo)
    h2 = h + _B_ref(_layernorm(h, axis=-1), B_w_gate, B_w_up, B_w_down)
    return h2
```

```python
import functools
import jax, jax.numpy as jnp
from jax import lax
from jax.experimental import pallas as pl
from jax.experimental.pallas import tpu as pltpu
S, D, H, DH, F = 2048, 512, 32, 16, 1792
C = (DH ** -0.5) * 1.4426950408889634
LMIN = 2.0 ** -40
bf, f32 = jnp.bfloat16, jnp.float32
def ln(x):
    m = jnp.mean(x, axis=-1, keepdims=True); xc = x - m
    v = jnp.mean(xc * xc, axis=-1, keepdims=True)
    return xc * lax.rsqrt(v + 1e-5)
def mm(a, b): return jnp.dot(a, b, preferred_element_type=f32)

def nt(a, b): return lax.dot_general(a, b, (((1,), (1,)), ((), ())), preferred_element_type=f32)
def lhs7(a11, a12, a21, a22):
    return [t.astype(bf) for t in (a11 + a22, a21 + a22, a11, a22, a11 + a12, a21 - a11, a12 - a22)]
def rhs5(b11, b12, b21, b22):
    b11, b12, b21, b22 = (t.astype(f32) for t in (b11, b12, b21, b22))
    return [t.astype(bf) for t in (b11 + b22, b12 - b22, b21 - b11, b11 + b12, b21 + b22)]
WI = {0: 0, 2: 1, 3: 2, 5: 3, 6: 4}
ORD = (2, 4, 3, 1, 5, 0, 6)
def comb(m):
    return m[3] - m[4] + m[0] + m[6], m[2] + m[4], m[1] + m[3], m[2] - m[1] + m[5] + m[0]
def kern(x_h, wqkv_h, wo_h, wg_h, wu_h, wd_h, o_h,
         x_s, wqkv_s, wo_s, wg_s, wu_s, wd_s, o_s, k_s, qt_s, vt_s, ot_s, b_s, s_s, w1_s, w2_s, kf_s, qf_s, kb_s, wt_s, xn_s, sem, osem,
         *, TQ, TK, TM, T1, HU, PL, DIV, NV, VB, FC, WP, VE, KG, PC, PD, PF):
    NQ = S // TQ
    xcp = [pltpu.make_async_copy(x_h.at[pl.ds(i * T1, T1)], x_s.at[pl.ds(i * T1, T1)], sem.at[7 + i]) for i in range(S // T1)]
    wcp = [pltpu.make_async_copy(wqkv_h.at[:, pl.ds(j * D, D)], wqkv_s.at[j], sem.at[j]) for j in range(3)]
    fcp = [pltpu.make_async_copy(a, b, sem.at[3 + j]) for j, (a, b) in enumerate(((wo_h, wo_s), (wg_h, wg_s), (wu_h, wu_s), (wd_h, wd_s)))]
    N1 = S // T1
    xcp[0].start(); wcp[0].start(); wcp[2].start(); wcp[1].start()
    xcp[0].wait(); xcp[1].start()
    xn_s[0] = ln(x_s[0:T1, :].astype(f32)).astype(bf)
    wcp[0].wait(); wt_s[0:D, :] = wqkv_s[0].T
    wcp[2].wait(); wt_s[D:2 * D, :] = wqkv_s[2].T
    for c in xcp[2:]: c.start()
    wcp[1].wait()
    lane = lax.broadcasted_iota(jnp.int32, (T1, 128), 1) % KG
    E = jnp.where(lax.broadcasted_iota(jnp.int32, (H, D), 1) // DH == lax.broadcasted_iota(jnp.int32, (H, D), 0), 1.0, 0.0).astype(bf)
    def p1(i, kn):
        r = pl.ds(pl.multiple_of(i * T1, T1), T1)
        i1 = jnp.minimum(i + 1, N1 - 1)
        r1 = pl.ds(pl.multiple_of(i1 * T1, T1), T1)
        @pl.when(i + 1 < N1)
        def _():
            pltpu.make_async_copy(x_h.at[r1], x_s.at[r1], sem.at[7 + i1]).wait()
        @pl.when(i == 1)
        def _():
            for c in fcp: c.start()
        xc = xn_s[i % 2]
        qv = nt(wt_s[...], xc)
        qt = qv[0:D] * C
        qt_s[i] = qt.astype(bf)
        if NV: qf_s[i, :, 0:DH, :] = qt.reshape(H, DH, T1)
        b_s[i] = mm(E, (qt * qt).astype(bf))
        vt_s[:, r] = qv[D:2 * D].astype(bf)
        k = mm(xc, wqkv_s[1])
        for g in range(4):
            kg = k[:, g * 128:(g + 1) * 128]
            ke = jnp.where(lane == DH, 1.0, kg).astype(bf)
            ko = jnp.where(lane == 0, 1.0, kg).astype(bf)
            for j in range(128 // KG):
                k_s[(g * (128 // KG) + j) * 2, r, :] = ke[:, KG * j:KG * (j + 1)]
                k_s[(g * (128 // KG) + j) * 2 + 1, r, :] = ko[:, KG * j:KG * (j + 1)]
            for j in range(T1 // TK):
                kf_s[g, pl.ds(pl.multiple_of((i * (T1 // TK) + j) * 16, 16), 16), :] = kg[j * TK:j * TK + 16]
        xn_s[(i + 1) % 2] = ln(x_s[r1, :].astype(f32)).astype(bf)
        return jnp.maximum(kn, nt(E, (k * k).astype(bf)))
    with jax.named_scope('P1'):
        kn = lax.fori_loop(0, N1, p1, jnp.zeros((H, T1), f32))
    for c in fcp: c.wait()
    kn = jnp.max(kn, axis=1, keepdims=True)
    @pl.loop(0, NQ)
    def _(i):
        b = (-jnp.sqrt(b_s[i] * kn)).astype(bf).astype(f32)
        for h in range(H):
            qf_s[i, h, DH:DH + 8, :] = jnp.broadcast_to(b[h:h + 1, :], (8, TQ))
    def make_q(h, q, bm):
        if KG == 2 * DH and isinstance(h, tuple):
            return h[0], jnp.concatenate([q, bm] if h[1] % 2 == 0 else [bm, q], axis=0)
        h = h[0] if isinstance(h, tuple) else h
        j = h % (KG // DH); z = jnp.zeros((DH, TQ), f32); q = q.astype(f32); bm = bm.astype(f32)
        blk = [jnp.where(j == 0, q, bm), jnp.where(j == 0, bm, jnp.where(j == 1, q, z))] + [jnp.where(j == t, q, z) for t in range(2, KG // DH)]
        return (h // (KG // DH)) * 2 + jnp.where(j == 0, 0, 1), jnp.concatenate(blk, axis=0).astype(bf)
    row = lax.broadcasted_iota(jnp.int32, (DH, TQ), 0)
    NM = (S - NV) // TK
    def valu_stream(h, qi, slot, out):
        bc = lambda d, c: jnp.broadcast_to(qf_s[qi, h, d:d + 1, c * 128:(c + 1) * 128], (VB, 128))
        for k0 in range(0, NV, VB):
            s = [bc(DH, c) for c in range(TQ // 128)]
            for d in range(DH):
                pace = yield
                kb = kb_s[slot, d, k0:k0 + VB, :]
                if pace is not None:
                    kb = jnp.maximum(kb, jnp.minimum(kb, jnp.concatenate([pace] * (VB // 8), axis=0)))
                s = [t + kb * bc(d, c) for c, t in enumerate(s)]
            p = jnp.exp2(jnp.concatenate(s, axis=1))
            out.append(p)
        yield
    NC = S // TK; nb = NV // 16
    VT = [-(-(b + 1) * NC // nb) - 1 for b in range(nb)]
    def make_kb(h, slot, d0, d1):
        kf = jnp.concatenate([kf_s[h // 8, 16 * c:16 * c + 16, :] for c in VT], axis=0)
        kf = pltpu.roll(kf, (128 - (h % 8) * DH) % 128, 1)
        for d in range(d0, d1):
            kb_s[slot, d] = jnp.broadcast_to(kf[:, d:d + 1], (NV, 128))
    make_kb(0, 0, 0, DH)
    def att(i, bad):
        work = []
        def wprep():
            n1 = D // 2 // (H // HU); n2 = 32 * HU; i2 = jnp.minimum(i, F // 2 // n2 - 1)
            ra = pl.ds(pl.multiple_of(i * n1, n1), n1); rb = pl.ds(pl.multiple_of(D // 2 + i * n1, n1), n1)
            for j, t in enumerate(rhs5(wg_s[ra, :], wu_s[ra, :], wg_s[rb, :], wu_s[rb, :])): w1_s[j, ra, :] = t
            ra = pl.ds(pl.multiple_of(i2 * n2, 16), n2); rb = pl.ds(pl.multiple_of(F // 2 + i2 * n2, 16), n2)
            for j, t in enumerate(rhs5(wd_s[ra, 0:D // 2], wd_s[ra, D // 2:D], wd_s[rb, 0:D // 2], wd_s[rb, D // 2:D])): w2_s[j, ra, :] = t
        for hu in range(HU):
            h = i * HU + hu
            hr = pl.ds(pl.multiple_of(h * DH, DH), DH)
            for qi in range(NQ):
                for c in range(NC):
                    work.append((hu, h, hr, qi, c, c * TK, c == 0, c == NC - 1))
        ps = []; ls = []; pf = []; l = acc = None
        for g in range(len(work) + PL):
            if g < len(work):
                hu, h, hr, qi, c, k0, fst, lst = work[g]
                if fst:
                    l = None
                    qm = qt_s[qi, hr, :]
                    bm = jnp.where(row == 0, qf_s[qi, h, DH:DH + 1, :], 0.0).astype(bf)
                    kix, qm = make_q((h, hu) if HU % 2 == 0 else h, qm, bm)
                    vout = []; vs = valu_stream(h, qi, hu % 2, vout); next(vs); done = 0
                    make_kb(jnp.minimum(h + 1, H - 1), (hu + 1) % 2, qi * DH // NQ, (qi + 1) * DH // NQ)
                v = 16 if c in VT else 0
                p = jnp.exp2(mm(k_s[kix, k0 + v:k0 + TK, :], qm))
                pf.append(p)
                tot = NV // VB * DH; npt = NC * 16
                while done < tot and done * npt < (c + 1) * 16 * tot:
                    pt = done * npt // tot - c * 16
                    pc = None
                    if len(pf) >= PC and done % PD == 0:
                        pt = pt * (pf[-PC].shape[0] // 8) // 16
                        pc = pf[-PC][8 * pt:8 * pt + 8, 0:128]
                    vs.send(pc); done += 1
                if v:
                    pv = vout[:16 // VB]; del vout[:16 // VB]
                    p = jnp.concatenate(pv + [p], axis=0)
                t = p.reshape(-1, 8, TQ)
                for j in list(range(v // 8, TK // 8)) + list(range(v // 8)):
                    l = t[j] if l is None else l + t[j]
                ls.append(l); ps.append(p if PF else p.astype(bf))
            if g == int(WP * len(work)): wprep()
            if g >= PL:
                _, h2, hr2, q2, _, k2, fst2, lst2 = work[g - PL]
                pt = ps[g - PL]
                a = mm(vt_s[hr2, k2:k2 + TK].astype(pt.dtype), pt)
                acc = a if fst2 else acc + a
                if lst2:
                    lt = jnp.sum(ls[g - PL], axis=0, keepdims=True)
                    ot_s[q2, hr2, :] = acc * (1.0 / lt)
                    bad = jnp.maximum(bad, jnp.where((lt >= LMIN) & (lt <= 1.0 / LMIN), 0.0, 1.0))
        return bad
    with jax.named_scope('ATT'):
        bad = lax.fori_loop(0, H // HU // DIV, att, jnp.zeros((1, TQ), f32))

    @pl.when(jnp.max(bad) > 0.0)
    def _():
        def item(t, _):
            qi = t // H; h = t % H
            hr = pl.ds(pl.multiple_of(h * DH, DH), DH)
            kix, qm = make_q(h, qt_s[qi, hr, :], jnp.zeros((DH, TQ), bf))
            def c1(c, m):
                r = pl.ds(pl.multiple_of(c * 256, 256), 256)
                s = mm(k_s[kix, r, :], qm)
                s_s[r, :] = s
                return jnp.maximum(m, jnp.max(s, axis=0, keepdims=True))
            m = lax.fori_loop(0, S // 256, c1, jnp.full((1, TQ), -jnp.inf, f32))
            p = jnp.exp2(s_s[...] - m)
            ot_s[qi, hr, :] = mm(vt_s[hr, :], p.astype(bf)) * (1.0 / jnp.sum(p, axis=0, keepdims=True))
        lax.fori_loop(0, H * NQ, item, None)

    h2 = TQ // 2; F2 = F // 2; D2 = D // 2
    def ocp(i, t):
        r = pl.ds(pl.multiple_of(i * TQ + t * h2, h2), h2)
        return pltpu.make_async_copy(o_s.at[r], o_h.at[r], osem.at[2 * i + t])
    def ffn(i, _):
        rr = [pl.ds(pl.multiple_of(i * TQ + t * h2, h2), h2) for t in range(2)]
        hh = [x_s[rr[t], :].astype(f32) + mm(ot_s[i, :, t * h2:(t + 1) * h2].T.astype(bf), wo_s[...]) for t in range(2)]
        hn = [ln(t) for t in hh]
        L = lhs7(hn[0][:, :D2], hn[0][:, D2:], hn[1][:, :D2], hn[1][:, D2:])
        def act(c0):
            cs = slice(c0, c0 + FC)
            w = lambda j: wg_s[0:D2, cs] if j == 1 else wu_s[D2:D, cs] if j == 4 else w1_s[WI[j], :, cs]
            gt, ut, gb, ub = comb({j: mm(L[j], w(j)) for j in ORD})
            gt = 0.5 * gt; gb = 0.5 * gb
            return (gt + gt * jnp.tanh(gt)) * ut, (gb + gb * jnp.tanh(gb)) * ub
        m = {}
        for c0 in range(0, F2, FC):
            a11, a21 = act(c0); a12, a22 = act(c0 + F2)
            cs = slice(c0, c0 + FC)
            w = lambda j: wd_s[cs, 0:D2] if j == 1 else wd_s[F2 + c0:F2 + c0 + FC, D2:D] if j == 4 else w2_s[WI[j], cs, :]
            for j, t in enumerate(lhs7(a11, a12, a21, a22)):
                t = mm(t, w(j)); m[j] = m[j] + t if j in m else t
        c11, c12, c21, c22 = comb(m)
        o_s[rr[0], :] = (hh[0] + jnp.concatenate([c11, c12], axis=1)).astype(bf)
        o_s[rr[1], :] = (hh[1] + jnp.concatenate([c21, c22], axis=1)).astype(bf)
        ocp(i, 0).start(); ocp(i, 1).start()
    with jax.named_scope('FFN'):
        lax.fori_loop(0, NQ, ffn, None)
    for i in range(NQ):
        ocp(i, 0).wait(); ocp(i, 1).wait()

def run(A_x, wqkv, wo, B_x, wg, wu, wd, TQ=512, TK=128, TM=256, HU=4, PL=2, DIV=1, NV=128, VB=8, FC=896, WP=1.0, PF=0, PC=2, PD=1, VE=0, KG=128, flags=None):
    V = pltpu.VMEM; NQ = S // TQ; nv = max(NV, 8)
    out = pl.pallas_call(functools.partial(kern, TQ=TQ, TK=TK, TM=TM, T1=TQ, HU=HU, PL=PL, DIV=DIV, NV=NV, VB=VB, FC=FC, WP=WP, PF=PF, PC=PC, PD=PD, VE=VE, KG=KG),
        out_shape=jax.ShapeDtypeStruct((S, D), bf),
        in_specs=[pl.BlockSpec(memory_space=pl.ANY)] * 6, out_specs=pl.BlockSpec(memory_space=pl.ANY),
        scratch_shapes=[V((S, D), bf), V((3, D, D), bf), V((D, D), bf), V((D, F), bf), V((D, F), bf), V((F, D), bf), V((S, D), bf),
                        V((2 * D // KG, S, KG), bf), V((NQ, D, TQ), bf), V((D, S), bf), V((NQ, D, TQ), f32), V((NQ, H, TQ), f32), V((S, TQ), f32),
                        V((5, D // 2, F), bf), V((5, F // 2, D // 2), bf), V((4, S // TK * 16, 128), f32), V((NQ, H, DH + 8, TQ), f32), V((2, DH, nv, 128), f32), V((2 * D, D), bf), V((2, TQ, D), bf),
                        pltpu.SemaphoreType.DMA((7 + NQ,)), pltpu.SemaphoreType.DMA((2 * NQ,))],
        compiler_params=pltpu.CompilerParams(vmem_limit_bytes=110 * 2**20, flags=flags),
    )(A_x.reshape(S, D), wqkv, wo, wg, wu, wd)
    return out.reshape(1, S, D)


@jax.jit
def pallas_sequential_preLN__softmax_full_mha__swiglu_ffn__prompt_kernel(A_x, A_wqkv, A_wo, B_x, B_w_gate, B_w_up, B_w_down):
    return run(A_x, A_wqkv, A_wo, B_x, B_w_gate, B_w_up, B_w_down, )
```

```python
import functools

import jax
import jax.numpy as jnp
from jax import lax
from jax.experimental import pallas as pl
from jax.experimental.pallas import tpu as pltpu

S, D, H, DH, F = 2048, 512, 32, 16, 1792
QSCALE = (DH ** -0.5) * 1.4426950408889634
LMIN, LMAX = 2.0 ** -80, 2.0 ** 40
TQ = 512
TK = 128
NQ, NC = S // TQ, S // TK
HG = 128 // DH
D2, F2, TH = D // 2, F // 2, TQ // 2
BF, F32 = jnp.bfloat16, jnp.float32
PRE = {0: 0, 2: 1, 3: 2, 4: 3, 6: 4}


def _ln(x):
    xc = x - jnp.mean(x, axis=-1, keepdims=True)
    return xc * lax.rsqrt(jnp.mean(xc * xc, axis=-1, keepdims=True) + 1e-5)


def _mm(a, b):
    return jnp.dot(a, b, preferred_element_type=F32)


def _mm_nt(a, b):
    return lax.dot_general(a, b, (((1,), (1,)), ((), ())), preferred_element_type=F32)


def _rows(start, size):
    return pl.ds(pl.multiple_of(start, size if size < 224 else 16), size)


def _strassen_lhs(a11, a12, a21, a22):
    return [t.astype(BF) for t in (a11, a11 + a12, a22, a11 + a22, a12 - a22, a21 + a22, a21 - a11)]


def _strassen_rhs(b11, b12, b21, b22):
    return [t.astype(BF) for t in (b12 - b22, b21 - b11, b11 + b22, b21 + b22, b11 + b12)]


def _strassen_out(m3, m5, m4, m1, m7, m2, m6):
    return m4 - m5 + m1 + m7, m3 + m5, m2 + m4, m3 + m1 - m2 + m6


def _q_operand(h, q, shift):
    j = h % HG
    q, shift, zero = q.astype(F32), shift.astype(F32), jnp.zeros((DH, TQ), F32)
    blocks = [jnp.where(j == 0, q, shift), jnp.where(j == 0, shift, jnp.where(j == 1, q, zero))]
    blocks += [jnp.where(j == t, q, zero) for t in range(2, HG)]
    return (h // HG) * 2 + jnp.where(j == 0, 0, 1), jnp.concatenate(blocks, axis=0).astype(BF)


def _kernel(x_h, wqkv_h, wo_h, wg_h, wu_h, wd_h, o_h,
            x_s, wk_s, wqv_s, wo_s, wg_s, wu_s, wd_s, o_s, k_s, qt_s, vt_s, ot_s, s_s, w1_s, w2_s,
            kf_s, qf_s, kb_s, wt_s, xn_s, xsem, wsem, fsem, osem, *, HU, NV, PL, SH, KB):
    WQ, n1, n2 = 2 * D // NQ, D2 // NQ, F2 // NQ
    nb = NV // 16
    vpu_tiles = [-(-(b + 1) * NC // nb) - 1 for b in range(nb)]

    xs = [(0, TH)] + [(TH + t * TQ, TQ) for t in range(NQ - 1)] + [(S - TH, TH)]
    x_cp = lambda t: pltpu.make_async_copy(x_h.at[pl.ds(*xs[t])], x_s.at[pl.ds(*xs[t])], xsem.at[t])
    wk_cp = pltpu.make_async_copy(wqkv_h.at[:, pl.ds(D, D)], wk_s, wsem.at[NQ])
    wo_cp = pltpu.make_async_copy(wo_h, wo_s, wsem.at[NQ + 1])

    def wqv_cp(i):
        cols = pl.ds(pl.multiple_of(i * WQ + (i // (NQ // 2)) * D, WQ), WQ)
        return pltpu.make_async_copy(wqkv_h.at[:, cols], wqv_s.at[i], wsem.at[i])

    def ffn_cps(i):
        parts = [(a, b, _rows(r * D2 + i * n1, n1)) for a, b in ((wg_h, wg_s), (wu_h, wu_s)) for r in range(2)]
        parts += [(wd_h, wd_s, _rows(r * F2 + i * n2, n2)) for r in range(2)]
        return [pltpu.make_async_copy(a.at[r], b.at[r], fsem.at[i]) for a, b, r in parts]

    x_cp(0).start(); wk_cp.start(); x_cp(1).start(); wqv_cp(0).start()
    x_cp(0).wait()
    xn_s[0:TH] = _ln(x_s[0:TH, :].astype(F32)).astype(BF)
    wk_cp.wait()
    lane = lax.broadcasted_iota(jnp.int32, (TQ, 128), 1)
    head_sum = jnp.where(lax.broadcasted_iota(jnp.int32, (H, D), 1) // DH
                         == lax.broadcasted_iota(jnp.int32, (H, D), 0), 1.0, 0.0).astype(BF)

    def phase_a(i, k2max):
        for t in range(NQ):
            pl.when(i == t)(x_cp(t + 1).wait)
        wqv_cp(i).wait()

        @pl.when(i == 0)
        def _():
            for t in range(1, NQ):
                x_cp(t + 1).start(); wqv_cp(t).start()

        @pl.when(i > 0)
        def _():
            for c in ffn_cps(i - 1):
                c.start()

        lower, ahead = _rows(i * TQ + TH, TH), _rows(jnp.minimum((i + 1) * TQ, S - TH), TH)
        xa = xn_s[_rows(i * TQ, TH), :]
        xb = _ln(x_s[lower, :].astype(F32)).astype(BF)
        k = jnp.concatenate([_mm(xa, wk_s[...]), _mm(xb, wk_s[...])], axis=0)
        xn_s[lower, :] = xb
        for g in range(H // HG):
            kg = k[:, g * 128:(g + 1) * 128]
            k_s[2 * g, _rows(i * TQ, TQ), :] = jnp.where(lane == DH, 1.0, kg).astype(BF)
            k_s[2 * g + 1, _rows(i * TQ, TQ), :] = jnp.where(lane == 0, 1.0, kg).astype(BF)
            for j in range(TQ // TK):
                kf_s[g, _rows((i * (TQ // TK) + j) * 16, 16), :] = kg[j * TK:j * TK + 16]
        wt_s[_rows(i * WQ, WQ), :] = wqv_s[i].T
        xn_s[ahead, :] = _ln(x_s[ahead, :].astype(F32)).astype(BF)
        return jnp.maximum(k2max, _mm_nt(head_sum, (k * k).astype(BF)))

    k2max = lax.fori_loop(0, NQ, phase_a, jnp.zeros((H, TQ), F32))
    for c in ffn_cps(NQ - 1):
        c.start()
    wo_cp.start()
    k2max = jnp.max(k2max, axis=1, keepdims=True)

    def bcast_k(g, lane0, slot, d0, n):
        kf = jnp.concatenate([kf_s[g, 16 * c:16 * c + 16, :] for c in vpu_tiles], axis=0)
        kf = pltpu.roll(kf, (128 - lane0) % 128, 1)
        for d in range(n):
            kb_s[slot, d0 + d] = jnp.broadcast_to(kf[:, d:d + 1], (NV, 128))

    def phase_b(i, _):
        for c in ffn_cps(i):
            c.wait()
        xc = xn_s[_rows(i * TQ, TQ), :]
        for t in range(2):
            y = _mm_nt(wt_s[t * D:(t + 1) * D, :], xc)
            if t == 0:
                q = y * QSCALE
                qt_s[i] = q.astype(BF)
                qf_s[i, :, 0:DH, :] = q.reshape(H, DH, TQ)
                shift = (-jnp.sqrt(_mm(head_sum, (q * q).astype(BF)) * k2max)).astype(BF).astype(F32)
                for h in range(H):
                    qf_s[i, h, DH:DH + 8, :] = jnp.broadcast_to(shift[h:h + 1, :], (8, TQ))
            else:
                vt_s[:, _rows(i * TQ, TQ)] = y.astype(BF)
            for c in range(7):
                paced = lambda w: jnp.where(
                    i >= 0, w, y[c * 64:c * 64 + w.shape[0], 0:w.shape[1]].astype(BF)).astype(F32)
                cols = slice((7 * t + c) * 128, (7 * t + c + 1) * 128)
                blk = [paced(w[_rows(r * D2 + i * n1, n1), cols]) for r in range(2) for w in (wg_s, wu_s)]
                for j, e in enumerate(_strassen_rhs(*blk)):
                    w1_s[j, _rows(i * n1, n1), cols] = e
                r0 = i * n2 + (7 * t + c) * 16
                blk = [paced(wd_s[_rows(r * F2 + r0, 16), u * D2:(u + 1) * D2]) for r in range(2) for u in range(2)]
                for j, e in enumerate(_strassen_rhs(*blk)):
                    w2_s[j, _rows(r0, 16), :] = e
        bcast_k(0, i * (DH // NQ), 0, i * (DH // NQ), DH // NQ)

    lax.fori_loop(0, NQ, phase_b, None)
    wo_cp.wait()

    def vpu_scores(h, qi, slot, out):
        q_row = lambda d, c: jnp.broadcast_to(qf_s[qi, h, d:d + 1, c * 128:(c + 1) * 128], (8, 128))
        keep = q_row(DH, 0) <= 0.0
        for k0 in range(0, NV, 8):
            s = [q_row(DH, c) for c in range(TQ // 128)]
            for d in range(DH):
                pace = yield
                kb = kb_s[slot, d, k0:k0 + 8, :]
                if pace is not None:
                    kb = jnp.where(keep, kb, pace)
                s = [t + kb * q_row(d, c) for c, t in enumerate(s)]
            out.append(jnp.exp2(jnp.concatenate(s, axis=1)))
        yield

    def add_rows(l, p):
        for j in range(0, p.shape[0], 8):
            l = p[j:j + 8] if l is None else l + p[j:j + 8]
        return l

    row = lax.broadcasted_iota(jnp.int32, (DH, TQ), 0)

    def attention(i, bad):
        vpu_p, pending, state = [], [], {"bad": bad}
        streams = [vpu_scores(i * HU + u, qi, u % 2, vpu_p) for u in range(HU) for qi in range(NQ)]
        steps, done, g = NV // 8 * DH, 0, 0

        def pv_step():
            feat, qi, c, p, l = pending.pop(0)
            a = _mm(vt_s[feat, c * TK:(c + 1) * TK], p)
            state["acc"] = a if c == 0 else state["acc"] + a
            if c == NC - 1:
                l = jnp.sum(l, axis=0, keepdims=True)
                ot_s[qi, feat, :] = (state["acc"] * (1.0 / l)).astype(BF)
                state["bad"] = jnp.maximum(state["bad"], jnp.where((l >= LMIN) & (l <= LMAX), 0.0, 1.0))

        for u in range(HU):
            h = i * HU + u
            feat = _rows(h * DH, DH)
            for qi in range(NQ):
                shift = jnp.where(row == 0, qf_s[qi, h, DH:DH + 1, :], 0.0)
                kix, qm = _q_operand(h, qt_s[qi, feat, :], shift)
                l = None
                for c in range(NC):
                    if c == KB:
                        h1, d0 = jnp.minimum(h + 1, H - 1), qi * (DH // NQ)
                        bcast_k(h1 // HG, (h1 % HG) * DH + d0, (u + 1) % 2, d0, DH // NQ)
                    skip = 16 if c in vpu_tiles else 0
                    p = jnp.exp2(_mm(k_s[kix, c * TK + skip:(c + 1) * TK, :], qm))
                    while done < steps * len(streams) and done * NC * 16 < ((g + 1) * 16 + SH) * steps:
                        r = (done * NC * 16 // steps - g * 16 - SH) * (p.shape[0] // 8) // 16
                        stream = streams[done // steps]
                        if done % steps == 0:
                            next(stream)
                        stream.send(p[8 * r:8 * r + 8, TQ - 128:TQ] if r >= 0 else None)
                        done += 1
                    g += 1
                    l = add_rows(l, p)
                    if skip:
                        extra = [vpu_p.pop(0), vpu_p.pop(0)]
                        for e in extra:
                            l = add_rows(l, e)
                        p = jnp.concatenate(extra + [p], axis=0)
                    pending.append((feat, qi, c, p.astype(BF), l))
                    if len(pending) > PL:
                        pv_step()
        while pending:
            pv_step()
        return state["bad"]

    bad = lax.fori_loop(0, H // HU, attention, jnp.zeros((1, TQ), F32))

    @pl.when(jnp.max(bad) > 0.0)
    def _():
        def true_max_attention(t, _):
            qi, h = t // H, t % H
            feat = _rows(h * DH, DH)
            kix, qm = _q_operand(h, qt_s[qi, feat, :], jnp.zeros((DH, TQ), F32))

            def scores(c, m):
                s = _mm(k_s[kix, _rows(c * 256, 256), :], qm)
                s_s[_rows(c * 256, 256), :] = s
                return jnp.maximum(m, jnp.max(s, axis=0, keepdims=True))

            m = lax.fori_loop(0, S // 256, scores, jnp.full((1, TQ), -jnp.inf, F32))
            p = jnp.exp2(s_s[...] - m)
            o = _mm(vt_s[feat, :], p.astype(BF)) * (1.0 / jnp.sum(p, axis=0, keepdims=True))
            ot_s[qi, feat, :] = o.astype(BF)

        lax.fori_loop(0, H * NQ, true_max_attention, None)

    def out_cp(i, t):
        r = _rows(i * TQ + t * TH, TH)
        return pltpu.make_async_copy(o_s.at[r], o_h.at[r], osem.at[2 * i + t])

    def ffn(i, _):
        half = [_rows(i * TQ + t * TH, TH) for t in range(2)]
        res = [x_s[half[t], :].astype(F32) + _mm(ot_s[i, :, t * TH:(t + 1) * TH].T, wo_s[...]) for t in range(2)]
        top, bot = _ln(res[0]), _ln(res[1])
        lhs = _strassen_lhs(top[:, :D2], top[:, D2:], bot[:, :D2], bot[:, D2:])

        def swiglu(cols):
            w = lambda j: wu_s[D2:D, cols] if j == 1 else wg_s[0:D2, cols] if j == 5 else w1_s[PRE[j], :, cols]
            gt, ut, gb, ub = _strassen_out(*[_mm(a, w(j)) for j, a in enumerate(lhs)])
            gt, gb = 0.5 * gt, 0.5 * gb
            return (gt + gt * jnp.tanh(gt)) * ut, (gb + gb * jnp.tanh(gb)) * ub

        a11, a21 = swiglu(slice(0, F2))
        a12, a22 = swiglu(slice(F2, F))
        w = lambda j: wd_s[F2:F, D2:D] if j == 1 else wd_s[0:F2, 0:D2] if j == 5 else w2_s[PRE[j]]
        y = _strassen_out(*[_mm(a, w(j)) for j, a in enumerate(_strassen_lhs(a11, a12, a21, a22))])
        for t in range(2):
            o_s[half[t], :] = (res[t] + jnp.concatenate(y[2 * t:2 * t + 2], axis=1)).astype(o_s.dtype)
            out_cp(i, t).start()

    lax.fori_loop(0, NQ, ffn, None)
    for i in range(NQ):
        out_cp(i, 0).wait(); out_cp(i, 1).wait()


def run(A_x, wqkv, wo, B_x, wg, wu, wd, HU=4, NV=160, PL=2, SH=6, KB=6):
    del B_x
    vmem, dma = pltpu.VMEM, pltpu.SemaphoreType.DMA
    out = pl.pallas_call(
        functools.partial(_kernel, HU=HU, NV=NV, PL=PL, SH=SH, KB=KB),
        out_shape=jax.ShapeDtypeStruct((S, D), A_x.dtype),
        in_specs=[pl.BlockSpec(memory_space=pl.ANY)] * 6,
        out_specs=pl.BlockSpec(memory_space=pl.ANY),
        scratch_shapes=[
            vmem((S, D), BF), vmem((D, D), BF), vmem((NQ, D, 2 * D // NQ), BF), vmem((D, D), BF),
            vmem((D, F), BF), vmem((D, F), BF), vmem((F, D), BF), vmem((S, D), A_x.dtype),
            vmem((2 * H // HG, S, 128), BF), vmem((NQ, D, TQ), BF), vmem((D, S), BF), vmem((NQ, D, TQ), BF),
            vmem((S, TQ), F32), vmem((5, D2, F), BF), vmem((5, F2, D2), BF),
            vmem((H // HG, NC * 16, 128), F32), vmem((NQ, H, DH + 8, TQ), F32), vmem((2, DH, NV, 128), F32),
            vmem((2 * D, D), BF), vmem((S, D), BF),
            dma((NQ + 1,)), dma((NQ + 2,)), dma((NQ,)), dma((2 * NQ,)),
        ],
        compiler_params=pltpu.CompilerParams(
            vmem_limit_bytes=100 * 2 ** 20,
            flags={"XLA_TPU_EVENLY_DISTRIBUTE_CRITICAL_NODES": True}),
    )(A_x.reshape(S, D), wqkv, wo, wg, wu, wd)
    return out.reshape(1, S, D)


@jax.jit
def pallas_sequential_preLN__softmax_full_mha__swiglu_ffn__prompt_kernel(A_x, A_wqkv, A_wo, B_x, B_w_gate, B_w_up, B_w_down):
    return run(A_x, A_wqkv, A_wo, B_x, B_w_gate, B_w_up, B_w_down)
```

```python
import functools

import jax
import jax.numpy as jnp
from jax import lax
from jax.experimental import pallas as pl
from jax.experimental.pallas import tpu as pltpu

S, D, H, DH, F = 2048, 512, 32, 16, 1792
QSCALE = (DH ** -0.5) * 1.4426950408889634
LMIN, LMAX = 2.0 ** -80, 2.0 ** 40
TQ = 512
TK = 128
NQ, NC = S // TQ, S // TK
HG = 128 // DH
D2, F2, TH = D // 2, F // 2, TQ // 2
BF, F32 = jnp.bfloat16, jnp.float32
PRE = {0: 0, 2: 1, 3: 2, 4: 3, 6: 4}


def _ln(x):
    xc = x - jnp.mean(x, axis=-1, keepdims=True)
    return xc * lax.rsqrt(jnp.mean(xc * xc, axis=-1, keepdims=True) + 1e-5)


def _mm(a, b):
    return jnp.dot(a, b, preferred_element_type=F32)


def _mm_nt(a, b):
    return lax.dot_general(a, b, (((1,), (1,)), ((), ())), preferred_element_type=F32)


def _rows(start, size):
    return pl.ds(pl.multiple_of(start, size if size < 224 else 16), size)


def _strassen_lhs(a11, a12, a21, a22):
    return [t.astype(BF) for t in (a11, a11 + a12, a22, a11 + a22, a12 - a22, a21 + a22, a21 - a11)]


def _strassen_rhs(b11, b12, b21, b22):
    return [t.astype(BF) for t in (b12 - b22, b21 - b11, b11 + b22, b21 + b22, b11 + b12)]


def _strassen_out(m3, m5, m4, m1, m7, m2, m6):
    return m4 - m5 + m1 + m7, m3 + m5, m2 + m4, m3 + m1 - m2 + m6


def _q_operand(h, q, shift):
    j = h % HG
    q, shift, zero = q.astype(F32), shift.astype(F32), jnp.zeros((DH, TQ), F32)
    blocks = [jnp.where(j == 0, q, shift), jnp.where(j == 0, shift, jnp.where(j == 1, q, zero))]
    blocks += [jnp.where(j == t, q, zero) for t in range(2, HG)]
    return (h // HG) * 2 + jnp.where(j == 0, 0, 1), jnp.concatenate(blocks, axis=0).astype(BF)


def _kernel(x_h, wqkv_h, wo_h, wg_h, wu_h, wd_h, o_h,
            x_s, wk_s, wqv_s, wo_s, wg_s, wu_s, wd_s, o_s, k_s, qt_s, vt_s, ot_s, s_s, w1_s, w2_s,
            kf_s, qf_s, kb_s, wt_s, xn_s, xsem, wsem, fsem, osem, *, HU, NV, PL, SH, KB, PN):
    WQ, n1, n2 = D // NQ, D2 // NQ, F2 // NQ
    nb = NV // 16
    vpu_tiles = [-(-(b + 1) * NC // nb) - 1 for b in range(nb)]

    xs = [(0, TH)] + [(TH + t * TQ, TQ) for t in range(NQ - 1)] + [(S - TH, TH)]
    x_cp = lambda t: pltpu.make_async_copy(x_h.at[pl.ds(*xs[t])], x_s.at[pl.ds(*xs[t])], xsem.at[t])
    wk_cp = pltpu.make_async_copy(wqkv_h.at[:, pl.ds(D, D)], wk_s, wsem.at[NQ])
    wo_cp = pltpu.make_async_copy(wo_h, wo_s, wsem.at[NQ + 1])

    def wqv_cps(i):
        cols = lambda t: pl.ds(pl.multiple_of(2 * t * D + i * WQ, WQ), WQ)
        return [pltpu.make_async_copy(wqkv_h.at[:, cols(t)], wqv_s.at[i, t], wsem.at[i]) for t in range(2)]

    def ffn_cps(i):
        parts = [(a, b, _rows(r * D2 + i * n1, n1)) for a, b in ((wg_h, wg_s), (wu_h, wu_s)) for r in range(2)]
        parts += [(wd_h, wd_s, _rows(r * F2 + i * n2, n2)) for r in range(2)]
        return [pltpu.make_async_copy(a.at[r], b.at[r], fsem.at[i]) for a, b, r in parts]

    x_cp(0).start(); wk_cp.start(); x_cp(1).start()
    for c in wqv_cps(0):
        c.start()
    x_cp(0).wait()
    xn_s[0:TH] = _ln(x_s[0:TH, :].astype(F32)).astype(BF)
    wk_cp.wait()
    lane = lax.broadcasted_iota(jnp.int32, (TQ, 128), 1)
    head_sum = jnp.where(lax.broadcasted_iota(jnp.int32, (H, D), 1) // DH
                         == lax.broadcasted_iota(jnp.int32, (H, D), 0), 1.0, 0.0).astype(BF)

    def phase_a(i, k2max):
        for t in range(NQ):
            pl.when(i == t)(x_cp(t + 1).wait)
        for c in wqv_cps(i):
            c.wait()

        @pl.when(i == 0)
        def _():
            for t in range(1, NQ):
                for c in [x_cp(t + 1)] + wqv_cps(t):
                    c.start()

        @pl.when(i > 0)
        def _():
            for c in ffn_cps(i - 1):
                c.start()

        lower, ahead = _rows(i * TQ + TH, TH), _rows(jnp.minimum((i + 1) * TQ, S - TH), TH)
        xa = xn_s[_rows(i * TQ, TH), :]
        xb = _ln(x_s[lower, :].astype(F32)).astype(BF)
        k = jnp.concatenate([_mm(xa, wk_s[...]), _mm(xb, wk_s[...])], axis=0)
        xn_s[lower, :] = xb
        for g in range(H // HG):
            kg = k[:, g * 128:(g + 1) * 128]
            k_s[2 * g, _rows(i * TQ, TQ), :] = jnp.where(lane == DH, 1.0, kg).astype(BF)
            k_s[2 * g + 1, _rows(i * TQ, TQ), :] = jnp.where(lane == 0, 1.0, kg).astype(BF)
            for j in range(TQ // TK):
                kf_s[g, _rows((i * (TQ // TK) + j) * 16, 16), :] = kg[j * TK:j * TK + 16]
        blk = [wqv_s[i, t, r * D2:(r + 1) * D2, :] for r in range(2) for t in range(2)]
        sums = _strassen_rhs(*[t.astype(F32) for t in blk])
        for j in range(7):
            wt_s[j, _rows(i * WQ, WQ), :] = (blk[3] if j == 1 else blk[0] if j == 5 else sums[PRE[j]]).T
        xn_s[ahead, :] = _ln(x_s[ahead, :].astype(F32)).astype(BF)
        return jnp.maximum(k2max, _mm_nt(head_sum, (k * k).astype(BF)))

    k2max = lax.fori_loop(0, NQ, phase_a, jnp.zeros((H, TQ), F32))
    for c in ffn_cps(NQ - 1):
        c.start()
    wo_cp.start()
    k2max = jnp.max(k2max, axis=1, keepdims=True)

    def bcast_k(g, lane0, slot, d0, n):
        kf = jnp.concatenate([kf_s[g, 16 * c:16 * c + 16, :] for c in vpu_tiles], axis=0)
        kf = pltpu.roll(kf, (128 - lane0) % 128, 1)
        for d in range(n):
            kb_s[slot, d0 + d] = jnp.broadcast_to(kf[:, d:d + 1], (NV, 128))

    def phase_b(i, _):
        for c in ffn_cps(i):
            c.wait()
        lhs = _strassen_lhs(*[xn_s[_rows(i * TQ + r * TH, TH), u * D2:(u + 1) * D2].astype(F32)
                              for r in range(2) for u in range(2)])
        m = [None] * 7
        for n, j in enumerate((2, 1, 3, 4, 5, 0, 6)):
            m[j] = _mm_nt(wt_s[j], lhs[j])
            for c in range(PN * n, min(PN * n + PN, 14)):
                paced = lambda w: jnp.where(i >= 0, w, m[j][
                    c % PN * 128:c % PN * 128 + w.shape[0], 0:w.shape[1]].astype(BF)).astype(F32)
                cols = slice(c * 128, (c + 1) * 128)
                blk = [paced(w[_rows(r * D2 + i * n1, n1), cols]) for r in range(2) for w in (wg_s, wu_s)]
                for t, e in enumerate(_strassen_rhs(*blk)):
                    w1_s[t, _rows(i * n1, n1), cols] = e
                r0 = i * n2 + c * 16
                blk = [paced(wd_s[_rows(r * F2 + r0, 16), u * D2:(u + 1) * D2]) for r in range(2) for u in range(2)]
                for t, e in enumerate(_strassen_rhs(*blk)):
                    w2_s[t, _rows(r0, 16), :] = e
        q_top, v_top, q_bot, v_bot = _strassen_out(*m)
        q = jnp.concatenate([q_top, q_bot], axis=1) * QSCALE
        qt_s[i] = q.astype(BF)
        qf_s[i, :, 0:DH, :] = q.reshape(H, DH, TQ)
        shift = (-jnp.sqrt(_mm(head_sum, (q * q).astype(BF)) * k2max)).astype(BF).astype(F32)
        for h in range(H):
            qf_s[i, h, DH:DH + 8, :] = jnp.broadcast_to(shift[h:h + 1, :], (8, TQ))
        vt_s[:, _rows(i * TQ, TQ)] = jnp.concatenate([v_top, v_bot], axis=1).astype(BF)
        bcast_k(0, i * (DH // NQ), 0, i * (DH // NQ), DH // NQ)

    lax.fori_loop(0, NQ, phase_b, None)
    wo_cp.wait()

    def vpu_scores(h, qi, slot, out):
        q_row = lambda d, c: jnp.broadcast_to(qf_s[qi, h, d:d + 1, c * 128:(c + 1) * 128], (8, 128))
        keep = q_row(DH, 0) <= 0.0
        for k0 in range(0, NV, 8):
            s = [q_row(DH, c) for c in range(TQ // 128)]
            for d in range(DH):
                pace = yield
                kb = kb_s[slot, d, k0:k0 + 8, :]
                if pace is not None:
                    kb = jnp.where(keep, kb, pace)
                s = [t + kb * q_row(d, c) for c, t in enumerate(s)]
            out.append(jnp.exp2(jnp.concatenate(s, axis=1)))
        yield

    def add_rows(l, p):
        for j in range(0, p.shape[0], 8):
            l = p[j:j + 8] if l is None else l + p[j:j + 8]
        return l

    row = lax.broadcasted_iota(jnp.int32, (DH, TQ), 0)

    def attention(i, bad):
        vpu_p, pending, state = [], [], {"bad": bad}
        streams = [vpu_scores(i * HU + u, qi, u % 2, vpu_p) for u in range(HU) for qi in range(NQ)]
        steps, done, g = NV // 8 * DH, 0, 0

        def pv_step():
            feat, qi, c, p, l = pending.pop(0)
            a = _mm(vt_s[feat, c * TK:(c + 1) * TK], p)
            state["acc"] = a if c == 0 else state["acc"] + a
            if c == NC - 1:
                l = jnp.sum(l, axis=0, keepdims=True)
                ot_s[qi, feat, :] = (state["acc"] * (1.0 / l)).astype(BF)
                state["bad"] = jnp.maximum(state["bad"], jnp.where((l >= LMIN) & (l <= LMAX), 0.0, 1.0))

        for u in range(HU):
            h = i * HU + u
            feat = _rows(h * DH, DH)
            for qi in range(NQ):
                shift = jnp.where(row == 0, qf_s[qi, h, DH:DH + 1, :], 0.0)
                kix, qm = _q_operand(h, qt_s[qi, feat, :], shift)
                l = None
                for c in range(NC):
                    if c == KB:
                        h1, d0 = jnp.minimum(h + 1, H - 1), qi * (DH // NQ)
                        bcast_k(h1 // HG, (h1 % HG) * DH + d0, (u + 1) % 2, d0, DH // NQ)
                    skip = 16 if c in vpu_tiles else 0
                    p = jnp.exp2(_mm(k_s[kix, c * TK + skip:(c + 1) * TK, :], qm))
                    while done < steps * len(streams) and done * NC * 16 < ((g + 1) * 16 + SH) * steps:
                        r = (done * NC * 16 // steps - g * 16 - SH) * (p.shape[0] // 8) // 16
                        stream = streams[done // steps]
                        if done % steps == 0:
                            next(stream)
                        stream.send(p[8 * r:8 * r + 8, TQ - 128:TQ] if r >= 0 else None)
                        done += 1
                    g += 1
                    l = add_rows(l, p)
                    if skip:
                        extra = [vpu_p.pop(0), vpu_p.pop(0)]
                        for e in extra:
                            l = add_rows(l, e)
                        p = jnp.concatenate(extra + [p], axis=0)
                    pending.append((feat, qi, c, p.astype(BF), l))
                    if len(pending) > PL:
                        pv_step()
        while pending:
            pv_step()
        return state["bad"]

    bad = lax.fori_loop(0, H // HU, attention, jnp.zeros((1, TQ), F32))

    @pl.when(jnp.max(bad) > 0.0)
    def _():
        def true_max_attention(t, _):
            qi, h = t // H, t % H
            feat = _rows(h * DH, DH)
            kix, qm = _q_operand(h, qt_s[qi, feat, :], jnp.zeros((DH, TQ), F32))

            def scores(c, m):
                s = _mm(k_s[kix, _rows(c * 256, 256), :], qm)
                s_s[_rows(c * 256, 256), :] = s
                return jnp.maximum(m, jnp.max(s, axis=0, keepdims=True))

            m = lax.fori_loop(0, S // 256, scores, jnp.full((1, TQ), -jnp.inf, F32))
            p = jnp.exp2(s_s[...] - m)
            o = _mm(vt_s[feat, :], p.astype(BF)) * (1.0 / jnp.sum(p, axis=0, keepdims=True))
            ot_s[qi, feat, :] = o.astype(BF)

        lax.fori_loop(0, H * NQ, true_max_attention, None)

    def out_cp(i, t):
        r = _rows(i * TQ + t * TH, TH)
        return pltpu.make_async_copy(o_s.at[r], o_h.at[r], osem.at[2 * i + t])

    def ffn(i, _):
        half = [_rows(i * TQ + t * TH, TH) for t in range(2)]
        res = [x_s[half[t], :].astype(F32) + _mm(ot_s[i, :, t * TH:(t + 1) * TH].T, wo_s[...]) for t in range(2)]
        top, bot = _ln(res[0]), _ln(res[1])
        lhs = _strassen_lhs(top[:, :D2], top[:, D2:], bot[:, :D2], bot[:, D2:])

        def swiglu(cols):
            w = lambda j: wu_s[D2:D, cols] if j == 1 else wg_s[0:D2, cols] if j == 5 else w1_s[PRE[j], :, cols]
            gt, ut, gb, ub = _strassen_out(*[_mm(a, w(j)) for j, a in enumerate(lhs)])
            gt, gb = 0.5 * gt, 0.5 * gb
            return (gt + gt * jnp.tanh(gt)) * ut, (gb + gb * jnp.tanh(gb)) * ub

        a11, a21 = swiglu(slice(0, F2))
        a12, a22 = swiglu(slice(F2, F))
        w = lambda j: wd_s[F2:F, D2:D] if j == 1 else wd_s[0:F2, 0:D2] if j == 5 else w2_s[PRE[j]]
        y = _strassen_out(*[_mm(a, w(j)) for j, a in enumerate(_strassen_lhs(a11, a12, a21, a22))])
        for t in range(2):
            o_s[half[t], :] = (res[t] + jnp.concatenate(y[2 * t:2 * t + 2], axis=1)).astype(o_s.dtype)
            out_cp(i, t).start()

    lax.fori_loop(0, NQ, ffn, None)
    for i in range(NQ):
        out_cp(i, 0).wait(); out_cp(i, 1).wait()


def run(A_x, wqkv, wo, B_x, wg, wu, wd, HU=4, NV=160, PL=2, SH=6, KB=6, PN=2):
    del B_x
    vmem, dma = pltpu.VMEM, pltpu.SemaphoreType.DMA
    out = pl.pallas_call(
        functools.partial(_kernel, HU=HU, NV=NV, PL=PL, SH=SH, KB=KB, PN=PN),
        out_shape=jax.ShapeDtypeStruct((S, D), A_x.dtype),
        in_specs=[pl.BlockSpec(memory_space=pl.ANY)] * 6,
        out_specs=pl.BlockSpec(memory_space=pl.ANY),
        scratch_shapes=[
            vmem((S, D), BF), vmem((D, D), BF), vmem((NQ, 2, D, D // NQ), BF), vmem((D, D), BF),
            vmem((D, F), BF), vmem((D, F), BF), vmem((F, D), BF), vmem((S, D), A_x.dtype),
            vmem((2 * H // HG, S, 128), BF), vmem((NQ, D, TQ), BF), vmem((D, S), BF), vmem((NQ, D, TQ), BF),
            vmem((S, TQ), F32), vmem((5, D2, F), BF), vmem((5, F2, D2), BF),
            vmem((H // HG, NC * 16, 128), F32), vmem((NQ, H, DH + 8, TQ), F32), vmem((2, DH, NV, 128), F32),
            vmem((7, D, D2), BF), vmem((S, D), BF),
            dma((NQ + 1,)), dma((NQ + 2,)), dma((NQ,)), dma((2 * NQ,)),
        ],
        compiler_params=pltpu.CompilerParams(
            vmem_limit_bytes=100 * 2 ** 20,
            flags={"XLA_TPU_EVENLY_DISTRIBUTE_CRITICAL_NODES": True}),
    )(A_x.reshape(S, D), wqkv, wo, wg, wu, wd)
    return out.reshape(1, S, D)


@jax.jit
def pallas_sequential_preLN__softmax_full_mha__swiglu_ffn__prompt_kernel(A_x, A_wqkv, A_wo, B_x, B_w_gate, B_w_up, B_w_down):
    return run(A_x, A_wqkv, A_wo, B_x, B_w_gate, B_w_up, B_w_down)
```

```python
import functools

import jax
import jax.numpy as jnp
from jax import lax
from jax.experimental import pallas as pl
from jax.experimental.pallas import tpu as pltpu

S, D, H, DH, F = 2048, 512, 32, 16, 1792
QSCALE = (DH ** -0.5) * 1.4426950408889634
LMIN, LMAX = 2.0 ** -80, 2.0 ** 40
TQ = 512
TK = 128
NQ, NC = S // TQ, S // TK
HG = 128 // DH
D2, F2, TH = D // 2, F // 2, TQ // 2
BF, F32 = jnp.bfloat16, jnp.float32
PRE = {0: 0, 2: 1, 3: 2, 4: 3, 6: 4}


def _ln(x):
    xc = x - jnp.mean(x, axis=-1, keepdims=True)
    return xc * lax.rsqrt(jnp.mean(xc * xc, axis=-1, keepdims=True) + 1e-5)


def _mm(a, b):
    return jnp.dot(a, b, preferred_element_type=F32)


def _mm_nt(a, b):
    return lax.dot_general(a, b, (((1,), (1,)), ((), ())), preferred_element_type=F32)


def _rows(start, size):
    return pl.ds(pl.multiple_of(start, size if size < 224 else 16), size)


def _strassen_lhs(a11, a12, a21, a22):
    return [t.astype(BF) for t in (a11, a11 + a12, a22, a11 + a22, a12 - a22, a21 + a22, a21 - a11)]


def _strassen_rhs(b11, b12, b21, b22):
    return [t.astype(BF) for t in (b12 - b22, b21 - b11, b11 + b22, b21 + b22, b11 + b12)]


def _strassen_out(m3, m5, m4, m1, m7, m2, m6):
    return m4 - m5 + m1 + m7, m3 + m5, m2 + m4, m3 + m1 - m2 + m6


def _q_operand(h, q, shift):
    j = h % HG
    q, shift, zero = q.astype(F32), shift.astype(F32), jnp.zeros((DH, TQ), F32)
    blocks = [jnp.where(j == 0, q, shift), jnp.where(j == 0, shift, jnp.where(j == 1, q, zero))]
    blocks += [jnp.where(j == t, q, zero) for t in range(2, HG)]
    return (h // HG) * 2 + jnp.where(j == 0, 0, 1), jnp.concatenate(blocks, axis=0).astype(BF)


def _kernel(x_h, wqkv_h, wo_h, wg_h, wu_h, wd_h, o_h,
            x_s, wk_s, wqv_s, wo_s, wg_s, wu_s, wd_s, o_s, k_s, qt_s, vt_s, ot_s, s_s, w1_s, w2_s, w3_s,
            kf_s, qf_s, kb_s, wt_s, xn_s, xsem, wsem, fsem, osem, *, HU, NV, PL, SH, KB, PN):
    WQ, n1, n2 = D // NQ, D2 // NQ, F2 // NQ
    nb = NV // 16
    vpu_tiles = [-(-(b + 1) * NC // nb) - 1 for b in range(nb)]

    xs = [(0, TH)] + [(TH + t * TQ, TQ) for t in range(NQ - 1)] + [(S - TH, TH)]
    x_cp = lambda t: pltpu.make_async_copy(x_h.at[pl.ds(*xs[t])], x_s.at[pl.ds(*xs[t])], xsem.at[t])
    wk_cp = pltpu.make_async_copy(wqkv_h.at[:, pl.ds(D, D)], wk_s, wsem.at[NQ])

    def wqv_cps(i):
        cols = lambda t: pl.ds(pl.multiple_of(2 * t * D + i * WQ, WQ), WQ)
        return [pltpu.make_async_copy(wqkv_h.at[:, cols(t)], wqv_s.at[i, t], wsem.at[i]) for t in range(2)]

    def ffn_cps(i):
        parts = [(a, b, _rows(r * D2 + i * n1, n1))
                 for a, b in ((wg_h, wg_s), (wu_h, wu_s), (wo_h, wo_s)) for r in range(2)]
        parts += [(wd_h, wd_s, _rows(r * F2 + i * n2, n2)) for r in range(2)]
        return [pltpu.make_async_copy(a.at[r], b.at[r], fsem.at[i]) for a, b, r in parts]

    x_cp(0).start(); wk_cp.start(); x_cp(1).start()
    for c in wqv_cps(0):
        c.start()
    x_cp(0).wait()
    xn_s[0:TH] = _ln(x_s[0:TH, :].astype(F32)).astype(BF)
    wk_cp.wait()
    lane = lax.broadcasted_iota(jnp.int32, (TQ, 128), 1)
    head_sum = jnp.where(lax.broadcasted_iota(jnp.int32, (H, D), 1) // DH
                         == lax.broadcasted_iota(jnp.int32, (H, D), 0), 1.0, 0.0).astype(BF)

    def phase_a(i, k2max):
        for t in range(NQ):
            pl.when(i == t)(x_cp(t + 1).wait)
        for c in wqv_cps(i):
            c.wait()

        @pl.when(i == 0)
        def _():
            for t in range(1, NQ):
                for c in [x_cp(t + 1)] + wqv_cps(t):
                    c.start()

        @pl.when(i > 0)
        def _():
            for c in ffn_cps(i - 1):
                c.start()

        lower, ahead = _rows(i * TQ + TH, TH), _rows(jnp.minimum((i + 1) * TQ, S - TH), TH)
        xa = xn_s[_rows(i * TQ, TH), :]
        xb = _ln(x_s[lower, :].astype(F32)).astype(BF)
        k = jnp.concatenate([_mm(xa, wk_s[...]), _mm(xb, wk_s[...])], axis=0)
        xn_s[lower, :] = xb
        for g in range(H // HG):
            kg = k[:, g * 128:(g + 1) * 128]
            k_s[2 * g, _rows(i * TQ, TQ), :] = jnp.where(lane == DH, 1.0, kg).astype(BF)
            k_s[2 * g + 1, _rows(i * TQ, TQ), :] = jnp.where(lane == 0, 1.0, kg).astype(BF)
            for j in range(TQ // TK):
                kf_s[g, _rows((i * (TQ // TK) + j) * 16, 16), :] = kg[j * TK:j * TK + 16]
        blk = [wqv_s[i, t, r * D2:(r + 1) * D2, :] for r in range(2) for t in range(2)]
        sums = _strassen_rhs(*[t.astype(F32) for t in blk])
        for j in range(7):
            wt_s[j, _rows(i * WQ, WQ), :] = (blk[3] if j == 1 else blk[0] if j == 5 else sums[PRE[j]]).T
        xn_s[ahead, :] = _ln(x_s[ahead, :].astype(F32)).astype(BF)
        return jnp.maximum(k2max, _mm_nt(head_sum, (k * k).astype(BF)))

    k2max = lax.fori_loop(0, NQ, phase_a, jnp.zeros((H, TQ), F32))
    for c in ffn_cps(NQ - 1):
        c.start()
    k2max = jnp.max(k2max, axis=1, keepdims=True)

    def bcast_k(g, lane0, slot, d0, n):
        kf = jnp.concatenate([kf_s[g, 16 * c:16 * c + 16, :] for c in vpu_tiles], axis=0)
        kf = pltpu.roll(kf, (128 - lane0) % 128, 1)
        for d in range(n):
            kb_s[slot, d0 + d] = jnp.broadcast_to(kf[:, d:d + 1], (NV, 128))

    def phase_b(i, _):
        for c in ffn_cps(i):
            c.wait()
        lhs = _strassen_lhs(*[xn_s[_rows(i * TQ + r * TH, TH), u * D2:(u + 1) * D2].astype(F32)
                              for r in range(2) for u in range(2)])
        m = [None] * 7
        for n, j in enumerate((2, 1, 3, 4, 5, 0, 6)):
            m[j] = _mm_nt(wt_s[j], lhs[j])
            for c in range(PN * n, min(PN * n + PN, 14)):
                paced = lambda w: jnp.where(i >= 0, w, m[j][
                    c % PN * 128:c % PN * 128 + w.shape[0], 0:w.shape[1]].astype(BF)).astype(F32)
                cols = slice(c * 128, (c + 1) * 128)
                blk = [paced(w[_rows(r * D2 + i * n1, n1), cols]) for r in range(2) for w in (wg_s, wu_s)]
                for t, e in enumerate(_strassen_rhs(*blk)):
                    w1_s[t, _rows(i * n1, n1), cols] = e
                if c < D2 // 128:
                    blk = [paced(wo_s[_rows(r * D2 + i * n1, n1), u * D2 + c * 128:u * D2 + (c + 1) * 128])
                           for r in range(2) for u in range(2)]
                    for t, e in enumerate(_strassen_rhs(*blk)):
                        w3_s[t, _rows(i * n1, n1), cols] = e
                r0 = i * n2 + c * 16
                blk = [paced(wd_s[_rows(r * F2 + r0, 16), u * D2:(u + 1) * D2]) for r in range(2) for u in range(2)]
                for t, e in enumerate(_strassen_rhs(*blk)):
                    w2_s[t, _rows(r0, 16), :] = e
        q_top, v_top, q_bot, v_bot = _strassen_out(*m)
        q = jnp.concatenate([q_top, q_bot], axis=1) * QSCALE
        qt_s[i] = q.astype(BF)
        qf_s[i, :, 0:DH, :] = q.reshape(H, DH, TQ)
        shift = (-jnp.sqrt(_mm(head_sum, (q * q).astype(BF)) * k2max)).astype(BF).astype(F32)
        for h in range(H):
            qf_s[i, h, DH:DH + 8, :] = jnp.broadcast_to(shift[h:h + 1, :], (8, TQ))
        vt_s[:, _rows(i * TQ, TQ)] = jnp.concatenate([v_top, v_bot], axis=1).astype(BF)
        bcast_k(0, i * (DH // NQ), 0, i * (DH // NQ), DH // NQ)

    lax.fori_loop(0, NQ, phase_b, None)

    def vpu_scores(h, qi, slot, out):
        q_row = lambda d, c: jnp.broadcast_to(qf_s[qi, h, d:d + 1, c * 128:(c + 1) * 128], (8, 128))
        keep = q_row(DH, 0) <= 0.0
        for k0 in range(0, NV, 8):
            s = [q_row(DH, c) for c in range(TQ // 128)]
            for d in range(DH):
                pace = yield
                kb = kb_s[slot, d, k0:k0 + 8, :]
                if pace is not None:
                    kb = jnp.where(keep, kb, pace)
                s = [t + kb * q_row(d, c) for c, t in enumerate(s)]
            out.append(jnp.exp2(jnp.concatenate(s, axis=1)))
        yield

    def add_rows(l, p):
        for j in range(0, p.shape[0], 8):
            l = p[j:j + 8] if l is None else l + p[j:j + 8]
        return l

    row = lax.broadcasted_iota(jnp.int32, (DH, TQ), 0)

    def attention(i, bad):
        vpu_p, pending, state = [], [], {"bad": bad}
        streams = [vpu_scores(i * HU + u, qi, u % 2, vpu_p) for u in range(HU) for qi in range(NQ)]
        steps, done, g = NV // 8 * DH, 0, 0

        def pv_step():
            feat, qi, c, p, l = pending.pop(0)
            a = _mm(vt_s[feat, c * TK:(c + 1) * TK], p)
            state["acc"] = a if c == 0 else state["acc"] + a
            if c == NC - 1:
                l = jnp.sum(l, axis=0, keepdims=True)
                ot_s[qi, feat, :] = (state["acc"] * (1.0 / l)).astype(BF)
                state["bad"] = jnp.maximum(state["bad"], jnp.where((l >= LMIN) & (l <= LMAX), 0.0, 1.0))

        for u in range(HU):
            h = i * HU + u
            feat = _rows(h * DH, DH)
            for qi in range(NQ):
                shift = jnp.where(row == 0, qf_s[qi, h, DH:DH + 1, :], 0.0)
                kix, qm = _q_operand(h, qt_s[qi, feat, :], shift)
                l = None
                for c in range(NC):
                    if c == KB:
                        h1, d0 = jnp.minimum(h + 1, H - 1), qi * (DH // NQ)
                        bcast_k(h1 // HG, (h1 % HG) * DH + d0, (u + 1) % 2, d0, DH // NQ)
                    skip = 16 if c in vpu_tiles else 0
                    p = jnp.exp2(_mm(k_s[kix, c * TK + skip:(c + 1) * TK, :], qm))
                    while done < steps * len(streams) and done * NC * 16 < ((g + 1) * 16 + SH) * steps:
                        r = (done * NC * 16 // steps - g * 16 - SH) * (p.shape[0] // 8) // 16
                        stream = streams[done // steps]
                        if done % steps == 0:
                            next(stream)
                        stream.send(p[8 * r:8 * r + 8, 256:384] if r >= 0 else None)
                        done += 1
                    g += 1
                    l = add_rows(l, p)
                    if skip:
                        extra = [vpu_p.pop(0), vpu_p.pop(0)]
                        for e in extra:
                            l = add_rows(l, e)
                        p = jnp.concatenate(extra + [p], axis=0)
                    pending.append((feat, qi, c, p.astype(BF), l))
                    if len(pending) > PL:
                        pv_step()
        while pending:
            pv_step()
        return state["bad"]

    bad = lax.fori_loop(0, H // HU, attention, jnp.zeros((1, TQ), F32))

    @pl.when(jnp.max(bad) > 0.0)
    def _():
        def true_max_attention(t, _):
            qi, h = t // H, t % H
            feat = _rows(h * DH, DH)
            kix, qm = _q_operand(h, qt_s[qi, feat, :], jnp.zeros((DH, TQ), F32))

            def scores(c, m):
                s = _mm(k_s[kix, _rows(c * 256, 256), :], qm)
                s_s[_rows(c * 256, 256), :] = s
                return jnp.maximum(m, jnp.max(s, axis=0, keepdims=True))

            m = lax.fori_loop(0, S // 256, scores, jnp.full((1, TQ), -jnp.inf, F32))
            p = jnp.exp2(s_s[...] - m)
            o = _mm(vt_s[feat, :], p.astype(BF)) * (1.0 / jnp.sum(p, axis=0, keepdims=True))
            ot_s[qi, feat, :] = o.astype(BF)

        lax.fori_loop(0, H * NQ, true_max_attention, None)

    def out_cp(i, t):
        r = _rows(i * TQ + t * TH, TH)
        return pltpu.make_async_copy(o_s.at[r], o_h.at[r], osem.at[2 * i + t])

    def ffn(i, _):
        half = [_rows(i * TQ + t * TH, TH) for t in range(2)]
        o = [ot_s[i, u * D2:(u + 1) * D2, t * TH:(t + 1) * TH].T.astype(F32) for t in range(2) for u in range(2)]
        w = lambda j: wo_s[D2:D, D2:D] if j == 1 else wo_s[0:D2, 0:D2] if j == 5 else w3_s[PRE[j]]
        y = _strassen_out(*[_mm(a, w(j)) for j, a in enumerate(_strassen_lhs(*o))])
        res = [x_s[half[t], :].astype(F32) + jnp.concatenate(y[2 * t:2 * t + 2], axis=1) for t in range(2)]
        top, bot = _ln(res[0]), _ln(res[1])
        lhs = _strassen_lhs(top[:, :D2], top[:, D2:], bot[:, :D2], bot[:, D2:])

        def swiglu(cols):
            w = lambda j: wu_s[D2:D, cols] if j == 1 else wg_s[0:D2, cols] if j == 5 else w1_s[PRE[j], :, cols]
            gt, ut, gb, ub = _strassen_out(*[_mm(a, w(j)) for j, a in enumerate(lhs)])
            gt, gb = 0.5 * gt, 0.5 * gb
            return (gt + gt * jnp.tanh(gt)) * ut, (gb + gb * jnp.tanh(gb)) * ub

        a11, a21 = swiglu(slice(0, F2))
        a12, a22 = swiglu(slice(F2, F))
        w = lambda j: wd_s[F2:F, D2:D] if j == 1 else wd_s[0:F2, 0:D2] if j == 5 else w2_s[PRE[j]]
        y = _strassen_out(*[_mm(a, w(j)) for j, a in enumerate(_strassen_lhs(a11, a12, a21, a22))])
        for t in range(2):
            o_s[half[t], :] = (res[t] + jnp.concatenate(y[2 * t:2 * t + 2], axis=1)).astype(o_s.dtype)
            out_cp(i, t).start()

    lax.fori_loop(0, NQ, ffn, None)
    for i in range(NQ):
        out_cp(i, 0).wait(); out_cp(i, 1).wait()


def run(A_x, wqkv, wo, B_x, wg, wu, wd, HU=4, NV=160, PL=2, SH=6, KB=6, PN=2):
    del B_x
    vmem, dma = pltpu.VMEM, pltpu.SemaphoreType.DMA
    out = pl.pallas_call(
        functools.partial(_kernel, HU=HU, NV=NV, PL=PL, SH=SH, KB=KB, PN=PN),
        out_shape=jax.ShapeDtypeStruct((S, D), A_x.dtype),
        in_specs=[pl.BlockSpec(memory_space=pl.ANY)] * 6,
        out_specs=pl.BlockSpec(memory_space=pl.ANY),
        scratch_shapes=[
            vmem((S, D), BF), vmem((D, D), BF), vmem((NQ, 2, D, D // NQ), BF), vmem((D, D), BF),
            vmem((D, F), BF), vmem((D, F), BF), vmem((F, D), BF), vmem((S, D), A_x.dtype),
            vmem((2 * H // HG, S, 128), BF), vmem((NQ, D, TQ), BF), vmem((D, S), BF), vmem((NQ, D, TQ), BF),
            vmem((S, TQ), F32), vmem((5, D2, F), BF), vmem((5, F2, D2), BF), vmem((5, D2, D2), BF),
            vmem((H // HG, NC * 16, 128), F32), vmem((NQ, H, DH + 8, TQ), F32), vmem((2, DH, NV, 128), F32),
            vmem((7, D, D2), BF), vmem((S, D), BF),
            dma((NQ + 1,)), dma((NQ + 1,)), dma((NQ,)), dma((2 * NQ,)),
        ],
        compiler_params=pltpu.CompilerParams(
            vmem_limit_bytes=100 * 2 ** 20,
            flags={"XLA_TPU_EVENLY_DISTRIBUTE_CRITICAL_NODES": True}),
    )(A_x.reshape(S, D), wqkv, wo, wg, wu, wd)
    return out.reshape(1, S, D)


@jax.jit
def pallas_sequential_preLN__softmax_full_mha__swiglu_ffn__prompt_kernel(A_x, A_wqkv, A_wo, B_x, B_w_gate, B_w_up, B_w_down):
    return run(A_x, A_wqkv, A_wo, B_x, B_w_gate, B_w_up, B_w_down)
```
